```python
import os as _os
_os.environ.setdefault("JAX_PLATFORMS", "cpu")
import jax
import jax.numpy as jnp

def _softmax(x, axis=-1):
    return jax.nn.softmax(x, axis=axis)
def _gelu(x):
    return jax.nn.gelu(x, approximate=True)
def _silu(x):
    return jax.nn.silu(x)
def _sigmoid(x):
    return jax.nn.sigmoid(x)
def _layernorm(x, axis=-1, eps=1e-5):
    m = jnp.mean(x, axis=axis, keepdims=True)
    v = jnp.var(x, axis=axis, keepdims=True)
    return (x - m) / jnp.sqrt(v + eps)
def _scatter_add(tgt, idx, src, axis=0):
    return tgt.at[idx].add(src)
def _segment_sum(src, seg, n):
    return jax.ops.segment_sum(src, seg, n)
class _Rng:
    def __init__(self, key):
        self._k = key
    def _next(self):
        self._k, sub = jax.random.split(self._k)
        return sub
    def normal(self, shape):
        return jax.random.normal(self._next(), shape, dtype=jnp.bfloat16)
    def randint(self, lo, hi, shape):
        return jax.random.randint(self._next(), shape, lo, hi, dtype=jnp.int32)
    def uniform(self, shape, lo=0.0, hi=1.0):
        return jax.random.uniform(self._next(), shape, jnp.bfloat16, lo, hi)
    def permutation(self, n):
        return jax.random.permutation(self._next(), n)


kernel_name = 'standalone__gqa_softmax__near_ridge'

def setup_inputs():
    _rng = _Rng(jax.random.key(int.from_bytes(__import__("os").urandom(4), "little")))
    _w = (lambda a: (lambda t: t.astype(jnp.bfloat16) if jnp.issubdtype(t.dtype, jnp.floating) else t)(jnp.asarray(a)))
    B, Hq, Hkv, Sq, Sk, D = 8, 16, 8, 512, 512, 256
    return {
        "q": _w((lambda *s: _rng.normal(s) * 0.4)(B, Hq, Sq, D)),
        "k": _w((lambda *s: _rng.normal(s) * 0.4)(B, Hkv, Sk, D)),
        "v": _w((lambda *s: _rng.normal(s) * 0.05)(B, Hkv, Sk, D)),
    }

def reference(q, k, v):
    B, Hq, Sq, D = q.shape
    Hkv = k.shape[1]
    rep = Hq // Hkv
    k = jnp.repeat(k, rep, axis=1)
    v = jnp.repeat(v, rep, axis=1)
    scale = D ** -0.5
    scores = jnp.einsum("bhqd,bhkd->bhqk", q, k) * scale
    p = _softmax(scores, axis=-1)
    return jnp.einsum("bhqk,bhkd->bhqd", p, v)
```

```python
import math

import jax
import jax.numpy as jnp
from jax import lax
import jax.experimental.pallas as pl
import jax.experimental.pallas.tpu as pltpu


@jax.jit
def pallas_standalone__gqa_softmax__near_ridge_kernel(
    q: jax.Array,
    k: jax.Array,
    v: jax.Array,
):
    B, Hq, Sq, D = q.shape
    Hkv, Sk = k.shape[1], k.shape[2]
    rep = Hq // Hkv
    N = B * Hkv
    M = rep * Sq
    c = D ** -0.5 * math.log2(math.e)

    def kernel_function(q_ref, k_ref, v_ref, o_ref):
        s = lax.dot_general(q_ref[...], k_ref[...], (((1,), (1,)), ((), ())),
                            preferred_element_type=jnp.float32)
        m = jnp.max(s, axis=-1, keepdims=True)
        p = jnp.exp2((s - m) * c)
        l = jnp.sum(p, axis=-1, keepdims=True)
        o = jnp.dot(p.astype(v_ref.dtype), v_ref[...], preferred_element_type=jnp.float32)
        o_ref[...] = (o * (1.0 / l)).astype(o_ref.dtype)

    out = pl.pallas_call(
        kernel_function,
        grid=(N,),
        in_specs=[
            pl.BlockSpec((None, M, D), lambda i: (i, 0, 0)),
            pl.BlockSpec((None, Sk, D), lambda i: (i, 0, 0)),
            pl.BlockSpec((None, Sk, D), lambda i: (i, 0, 0)),
        ],
        out_specs=pl.BlockSpec((None, M, D), lambda i: (i, 0, 0)),
        out_shape=jax.ShapeDtypeStruct((N, M, D), q.dtype),
        compiler_params=pltpu.CompilerParams(
            dimension_semantics=("parallel",),
            vmem_limit_bytes=64 * 1024 * 1024,
        ),
    )(q.reshape(N, M, D), k.reshape(N, Sk, D), v.reshape(N, Sk, D))
    return out.reshape(B, Hq, Sq, D)
```

```python
import functools
import math

import jax
import jax.numpy as jnp
from jax import lax
import jax.experimental.pallas as pl
import jax.experimental.pallas.tpu as pltpu

UNROLL = 16
PREFETCH = 2
PIECES = 4


def _attention_kernel(
    q_hbm, k_hbm, v_hbm, o_hbm, buf, q_sem, k_sem, v_sem, o_sem, *, unroll
):
    n_heads, q_rows, d = q_hbm.shape
    kv_rows = k_hbm.shape[1]
    k_off, v_off = q_rows, q_rows + kv_rows
    n_steps = n_heads // unroll
    c = d**-0.5 * math.log2(math.e)

    def q_copies(head, slot):
        pieces = PIECES if slot == 0 else 1
        rows = q_rows // pieces
        return [
            pltpu.make_async_copy(
                q_hbm.at[head, pl.ds(i * rows, rows)],
                buf.at[head, pl.ds(i * rows, rows)],
                q_sem.at[slot if i == 0 else unroll + i - 1],
            )
            for i in range(pieces)
        ]

    def k_copy(head, slot):
        return pltpu.make_async_copy(
            k_hbm.at[head], buf.at[head, pl.ds(k_off, kv_rows)], k_sem.at[slot]
        )

    def v_copy(head, slot):
        return pltpu.make_async_copy(
            v_hbm.at[head], buf.at[head, pl.ds(v_off, kv_rows)], v_sem.at[slot]
        )

    def fetch(head, slot):
        k_copy(head, slot).start()
        for copy in q_copies(head, slot):
            copy.start()
        v_copy(head, slot).start()

    for slot in range(PREFETCH):
        fetch(slot, slot)

    @pl.loop(0, n_steps)
    def _(step):
        for slot in range(unroll):
            head = step * unroll + slot

            if slot == 0:
                k_copy(head, slot).wait()
                rows = q_rows // PIECES
                q = []
                for i, copy in enumerate(q_copies(head, slot)):
                    copy.wait()
                    if i == 0:
                        k = buf[head, pl.ds(k_off, kv_rows), :]
                    q.append(buf[head, pl.ds(i * rows, rows), :])
                q = jnp.concatenate(q, axis=0)
            else:
                k = buf[head, pl.ds(k_off, kv_rows), :]
                q = buf[head, pl.ds(0, q_rows), :]

            s = lax.dot_general(
                q, k, (((1,), (1,)), ((), ())), preferred_element_type=jnp.float32
            )
            m = jnp.max(s, axis=-1, keepdims=True)
            p = jnp.exp2(s * c - m * c)
            l = jnp.sum(p, axis=-1, keepdims=True)

            v_copy(head, slot).wait()
            ahead = slot + PREFETCH
            if ahead < unroll:
                fetch(head + PREFETCH, ahead)
            else:
                pl.when(step < n_steps - 1)(
                    functools.partial(fetch, head + PREFETCH, ahead - unroll)
                )
            v = buf[head, pl.ds(v_off, kv_rows), :]
            if slot + 1 < unroll:
                k_copy(head + 1, slot + 1).wait()
                q_copies(head + 1, slot + 1)[0].wait()

            o = jnp.dot(p.astype(v.dtype), v, preferred_element_type=jnp.float32)
            o = (o * pltpu.reciprocal(l, full_range=False)).astype(buf.dtype)

            pieces = PIECES if slot == unroll - 1 else 1
            rows = q_rows // pieces
            for i in range(pieces):
                buf[head, pl.ds(i * rows, rows), :] = o[i * rows : (i + 1) * rows]
                pltpu.make_async_copy(
                    buf.at[head, pl.ds(i * rows, rows)],
                    o_hbm.at[head, pl.ds(i * rows, rows)],
                    o_sem,
                ).start()

    pltpu.make_async_copy(o_hbm, o_hbm, o_sem).wait()


@jax.jit
def pallas_standalone__gqa_softmax__near_ridge_kernel(
    q: jax.Array,
    k: jax.Array,
    v: jax.Array,
):
    b, hq, sq, d = q.shape
    hkv, sk = k.shape[1], k.shape[2]
    n_heads = b * hkv
    q_rows = (hq // hkv) * sq
    unroll = math.gcd(n_heads, UNROLL)
    assert PREFETCH < unroll and q.dtype == k.dtype == v.dtype

    out = pl.pallas_call(
        functools.partial(_attention_kernel, unroll=unroll),
        in_specs=[pl.BlockSpec(memory_space=pl.ANY)] * 3,
        out_specs=pl.BlockSpec(memory_space=pl.ANY),
        out_shape=jax.ShapeDtypeStruct((n_heads, q_rows, d), q.dtype),
        scratch_shapes=[
            pltpu.VMEM((n_heads, q_rows + 2 * sk, d), q.dtype),
            pltpu.SemaphoreType.DMA((unroll + PIECES - 1,)),
            pltpu.SemaphoreType.DMA((unroll,)),
            pltpu.SemaphoreType.DMA((unroll,)),
            pltpu.SemaphoreType.DMA(()),
        ],
        compiler_params=pltpu.CompilerParams(
            vmem_limit_bytes=100 * 1024 * 1024,
            disable_bounds_checks=True,
            flags={"XLA_TPU_RESCHEDULE_DMA_DONES": True},
        ),
    )(
        q.reshape(n_heads, q_rows, d),
        k.reshape(n_heads, sk, d),
        v.reshape(n_heads, sk, d),
    )
    return out.reshape(b, hq, sq, d)
```

```python
import functools
import math

import jax
import jax.numpy as jnp
from jax import lax
import jax.experimental.pallas as pl
import jax.experimental.pallas.tpu as pltpu

UNROLL = 16
PREFETCH = 2
Q_PIECES = 2
OUT_PIECE_ROWS = 32


def _attention_kernel(
    q_hbm, k_hbm, v_hbm, o_hbm, buf, q_sem, k_sem, v_sem, o_sem, *, unroll
):
    n_heads, q_rows, d = q_hbm.shape
    kv_rows = k_hbm.shape[1]
    k_rows = pl.ds(q_rows, kv_rows)
    v_rows = pl.ds(q_rows + kv_rows, kv_rows)
    n_steps = n_heads // unroll
    c = d**-0.5 * math.log2(math.e)

    def q_pieces(slot):
        n = Q_PIECES if slot == 0 else 1
        return [pl.ds(i * (q_rows // n), q_rows // n) for i in range(n)]

    def q_copy(head, slot, i=0):
        rows = q_pieces(slot)[i]
        sem = q_sem.at[slot % PREFETCH if i == 0 else PREFETCH + i - 1]
        return pltpu.make_async_copy(q_hbm.at[head, rows], buf.at[head, rows], sem)

    def k_copy(head, slot):
        return pltpu.make_async_copy(
            k_hbm.at[head], buf.at[head, k_rows], k_sem.at[slot % PREFETCH]
        )

    def v_copy(head, slot):
        return pltpu.make_async_copy(
            v_hbm.at[head], buf.at[head, v_rows], v_sem.at[slot % PREFETCH]
        )

    def fetch(head, slot):
        k_copy(head, slot).start()
        for i in range(len(q_pieces(slot))):
            q_copy(head, slot, i).start()
        v_copy(head, slot).start()

    for slot in range(PREFETCH):
        fetch(slot, slot)

    @pl.loop(0, n_steps)
    def _(step):
        k_copy(step * unroll, 0).wait()
        q_copy(step * unroll, 0).wait()

        for slot in range(unroll):
            head = step * unroll + slot

            k = buf[head, k_rows, :]
            q = []
            for i, rows in enumerate(q_pieces(slot)):
                if i > 0:
                    q_copy(head, slot, i).wait()
                q.append(buf[head, rows, :])
            q = jnp.concatenate(q, axis=0)

            s = lax.dot_general(
                q, k, (((1,), (1,)), ((), ())), preferred_element_type=jnp.float32
            )
            m = jnp.max(s, axis=-1, keepdims=True)
            p = jnp.exp2(s * c - m * c)
            l = jnp.sum(p, axis=-1, keepdims=True)

            v_copy(head, slot).wait()
            ahead = slot + PREFETCH
            if ahead < unroll:
                fetch(head + PREFETCH, ahead)
            else:
                pl.when(step < n_steps - 1)(
                    functools.partial(fetch, head + PREFETCH, ahead - unroll)
                )
            v = buf[head, v_rows, :]
            if slot + 1 < unroll:
                k_copy(head + 1, slot + 1).wait()
                q_copy(head + 1, slot + 1).wait()

            o = jnp.dot(p.astype(v.dtype), v, preferred_element_type=jnp.float32)
            o = (o * pltpu.reciprocal(l, full_range=False)).astype(buf.dtype)

            piece = OUT_PIECE_ROWS if slot == unroll - 1 else q_rows
            for start in range(0, q_rows, piece):
                rows = pl.ds(start, piece)
                buf[head, rows, :] = o[start : start + piece]
                pltpu.make_async_copy(
                    buf.at[head, rows], o_hbm.at[head, rows], o_sem
                ).start()

    pltpu.make_async_copy(o_hbm, o_hbm, o_sem).wait()


@jax.jit
def pallas_standalone__gqa_softmax__near_ridge_kernel(
    q: jax.Array,
    k: jax.Array,
    v: jax.Array,
):
    b, hq, sq, d = q.shape
    hkv, sk = k.shape[1], k.shape[2]
    n_heads = b * hkv
    q_rows = (hq // hkv) * sq
    unroll = math.gcd(n_heads, UNROLL)
    assert unroll > PREFETCH and unroll % PREFETCH == 0
    assert q_rows % (Q_PIECES * OUT_PIECE_ROWS) == 0
    assert q.dtype == k.dtype == v.dtype

    out = pl.pallas_call(
        functools.partial(_attention_kernel, unroll=unroll),
        in_specs=[pl.BlockSpec(memory_space=pl.ANY)] * 3,
        out_specs=pl.BlockSpec(memory_space=pl.ANY),
        out_shape=jax.ShapeDtypeStruct((n_heads, q_rows, d), q.dtype),
        scratch_shapes=[
            pltpu.VMEM((n_heads, q_rows + 2 * sk, d), q.dtype),
            pltpu.SemaphoreType.DMA((PREFETCH + Q_PIECES - 1,)),
            pltpu.SemaphoreType.DMA((PREFETCH,)),
            pltpu.SemaphoreType.DMA((PREFETCH,)),
            pltpu.SemaphoreType.DMA(()),
        ],
        compiler_params=pltpu.CompilerParams(
            vmem_limit_bytes=100 * 1024 * 1024,
            disable_bounds_checks=True,
            flags={"XLA_TPU_RESCHEDULE_DMA_DONES": True},
        ),
    )(
        q.reshape(n_heads, q_rows, d),
        k.reshape(n_heads, sk, d),
        v.reshape(n_heads, sk, d),
    )
    return out.reshape(b, hq, sq, d)
```
